```python
import jax
import jax.numpy as jnp

def _softmax(x, axis=-1):
    return jax.nn.softmax(x, axis=axis)
def _gelu(x):
    return jax.nn.gelu(x, approximate=True)
def _silu(x):
    return jax.nn.silu(x)
def _sigmoid(x):
    return jax.nn.sigmoid(x)
def _layernorm(x, axis=-1, eps=1e-5):
    m = jnp.mean(x, axis=axis, keepdims=True)
    v = jnp.var(x, axis=axis, keepdims=True)
    return (x - m) / jnp.sqrt(v + eps)
def _scatter_add(tgt, idx, src, axis=0):
    return tgt.at[idx].add(src)
def _segment_sum(src, seg, n):
    return jax.ops.segment_sum(src, seg, n)
class _Rng:
    def __init__(self, key):
        self._k = key
    def _next(self):
        self._k, sub = jax.random.split(self._k)
        return sub
    def normal(self, shape):
        return jax.random.normal(self._next(), shape, dtype=jnp.bfloat16)
    def randint(self, lo, hi, shape):
        return jax.random.randint(self._next(), shape, lo, hi, dtype=jnp.int32)
    def uniform(self, shape, lo=0.0, hi=1.0):
        return jax.random.uniform(self._next(), shape, jnp.bfloat16, lo, hi)
    def permutation(self, n):
        return jax.random.permutation(self._next(), n)


kernel_name = 'recurrent_scan__ssm_conv_h3__mixer_token_mlp__prompt'

def setup_inputs():
    _rng = _Rng(jax.random.key(int.from_bytes(__import__("os").urandom(4), "little")))
    _w = (lambda a: (lambda t: t.astype(jnp.bfloat16) if jnp.issubdtype(t.dtype, jnp.floating) else t)(jnp.asarray(a)))
    def _A_setup():
        B, S, D = 1, 2048, 576
        ks = 4
        return {
            "q": _w((lambda *s: _rng.normal(s) * 0.05)(B, S, D)),
            "k": _w((lambda *s: _rng.normal(s) * 0.05)(B, S, D)),
            "v": _w((lambda *s: _rng.normal(s) * 0.05)(B, S, D)),
            "shift_k": _w((lambda *s: _rng.normal(s) * 0.05)(D, ks) * 0.5),
            "ssm_k": _w((lambda *s: _rng.normal(s) * 0.05)(D, S) * (1.0 / S ** 0.5)),
            "ssm_D": _w((lambda *s: _rng.normal(s) * 0.05)(D)),
        }
    _A_in = _A_setup()

    def _B_setup():
        B, S, D, F = 1, 2048, 576, 4608
        return {
            "x": _w((lambda *s: _rng.normal(s) * 0.05)(B, S, D)),
            "w1": _w((lambda *s: _rng.normal(s) * 0.05)(S, F) * (S ** -0.5)),
            "b1": _w((lambda *s: _rng.normal(s) * 0.05)(F) * 0.02),
            "w2": _w((lambda *s: _rng.normal(s) * 0.05)(F, S) * (F ** -0.5)),
            "b2": _w((lambda *s: _rng.normal(s) * 0.05)(S) * 0.02),
        }
    _B_in = _B_setup()

    return {
        "A_q": _A_in["q"],
        "A_k": _A_in["k"],
        "A_v": _A_in["v"],
        "A_shift_k": _A_in["shift_k"],
        "A_ssm_k": _A_in["ssm_k"],
        "A_ssm_D": _A_in["ssm_D"],
        "B_x": _B_in["x"],
        "B_w1": _B_in["w1"],
        "B_b1": _B_in["b1"],
        "B_w2": _B_in["w2"],
        "B_b2": _B_in["b2"],
    }

def reference(A_q, A_k, A_v, A_shift_k, A_ssm_k, A_ssm_D, B_x, B_w1, B_b1, B_w2, B_b2):
    def _A_ref(q, k, v, shift_k, ssm_k, ssm_D):
        B, S, D = q.shape
        ks = shift_k.shape[-1]
        k_pad = jnp.pad(k, ((0, 0), (ks - 1, 0), (0, 0)))
        k_shift = jnp.zeros_like(k)
        for t in range(ks):
            k_shift = k_shift + k_pad[:, t:t + S, :] * shift_k[:, ks - 1 - t][None, None, :]
        kv = k_shift * v
        L = 2 * S
        kv_pad = jnp.pad(kv, ((0, 0), (0, S), (0, 0)))
        kf_pad = jnp.pad(ssm_k, ((0, 0), (0, S)))
        kv_f = (lambda x, axes=(-2,-1): jnp.fft.rfft2(x.astype(jnp.float32), axes=axes))(kv_pad[:, None, :, :], axes=(1, 2))
        kf_f = (lambda x, axes=(-2,-1): jnp.fft.rfft2(x.astype(jnp.float32), axes=axes))(kf_pad[:, None, :], axes=(1, 2))
        kf_f = (lambda x, *d: x.transpose(*d))(kf_f, 1, 2, 0)
        y_f = kv_f * kf_f[None, :, :, :]
        y = (lambda x, s, axes=(-2,-1): jnp.fft.irfft2(x, s=s, axes=axes).astype(jnp.bfloat16))(y_f, (1, L), axes=(1, 2))[:, 0, :S, :]
        y = y + kv * ssm_D[None, None, :]
        return q * y

    def _B_ref(x, w1, b1, w2, b2):
        B, S, D = x.shape
        h = _layernorm(x, axis=-1)
        u = jnp.einsum("bsd,sf->bdf", h, w1) + b1
        u = _gelu(u)
        y = jnp.einsum("bdf,fs->bds", u, w2) + b2
        return (lambda x, *d: x.transpose(*d))(y, 0, 2, 1)

    x = A_q
    xn = _layernorm(x, axis=-1)
    s = _A_ref(xn, A_k, A_v, A_shift_k, A_ssm_k, A_ssm_D)
    g = _silu(_B_ref(xn, B_w1, B_b1, B_w2, B_b2))
    return x + s * g
```

```python
import functools
import numpy as np
import jax, jax.numpy as jnp
from jax.experimental import pallas as pl
from jax.experimental.pallas import tpu as pltpu

S, D, F = 2048, 576, 4608
P = 128; A = S // P
f32, bf16 = jnp.float32, jnp.bfloat16

def _dft_consts():
    r = np.arange(P, dtype=np.float64)[:, None]
    f = np.arange(P, dtype=np.float64)[None, :]
    th = np.pi * (2 * f + 1) / (2 * P)
    Ft = np.concatenate([np.cos(th * r), -np.sin(th * r)], axis=1)
    G = Ft.T / P
    return Ft.astype(jnp.bfloat16), np.ascontiguousarray(G).astype(jnp.bfloat16)
FT_NP, G_NP = _dft_consts()

def gelu(x):
    c = 0.7978845608028654
    return 0.5 * x * (1.0 + jnp.tanh(c * (x + 0.044715 * x * x * x)))

def ln0(x):
    m = jnp.sum(x, axis=0, keepdims=True) * (1.0 / D)
    xc = x - m
    v = jnp.sum(xc * xc, axis=0, keepdims=True) * (1.0 / D)
    return xc * jax.lax.rsqrt(v + 1e-5)

def make(FC=512, NC=256, CG=64, QC=512, LNC=256, RG=16, AG=1, scopes=False, conv=True, KB=1, W2E=2, flags=None, alias=True, late=2):
    NJ = F // FC; NN = S // NC; NQ = S // QC; NG = D // CG
    assert NG == NJ
    import contextlib
    def scope(n):
        return jax.named_scope(n) if scopes else contextlib.nullcontext()

    def kernel(q_hbm, k_hbm, v_hbm, shift_ref, ssm_hbm, dd_ref, w1_hbm, b1_ref, w2_hbm, b2_ref,
               ft_ref, g_ref, o_hbm,
               xT, k_buf, v_buf, ssm_buf, w1_buf, w2a_buf, w2b_buf,
               xnT, hT, kvT, y_ref, u_ref, out_buf, wk_ref, pre_ref, zero_ref, col_ref, acc_ref,
               sem_q, sem_k, sem_v, sem_ssm, sem_w1, sem_w1p, sem_w2, sem_o):
        def q_copy(i):
            off = pl.multiple_of(i * QC, QC)
            return pltpu.make_async_copy(q_hbm.at[0, :, pl.ds(off, QC)], xT.at[:, pl.ds(off, QC)], sem_q.at[i])
        def w1_copy(j):
            off = pl.multiple_of(j * FC, FC)
            return pltpu.make_async_copy(w1_hbm.at[:, pl.ds(off, FC)], w1_buf.at[:, pl.ds(off, FC)], sem_w1.at[j])
        def w1p_copy(c):
            off = pl.multiple_of(c * QC, QC)
            return pltpu.make_async_copy(w1_hbm.at[pl.ds(off, QC), pl.ds(0, FC)], w1_buf.at[pl.ds(off, QC), pl.ds(0, FC)], sem_w1p.at[c])
        KH = F // 2
        def w2_copy(n, h):
            off = pl.multiple_of(n * NC, NC)
            return pltpu.make_async_copy(w2_hbm.at[pl.ds(h * KH, KH), pl.ds(off, NC)], (w2a_buf, w2b_buf)[h].at[:, pl.ds(off, NC)], sem_w2.at[2 * n + h])
        def grp_copy(hbm, buf, sem, g, three_d):
            off = pl.multiple_of(g * CG, CG)
            src = hbm.at[0, pl.ds(off, CG), :] if three_d else hbm.at[pl.ds(off, CG), :]
            return pltpu.make_async_copy(src, buf.at[pl.ds(off, CG), :], sem.at[g])
        k_copy = lambda g: grp_copy(k_hbm, k_buf, sem_k, g, True)
        v_copy = lambda g: grp_copy(v_hbm, v_buf, sem_v, g, True)
        ssm_copy = lambda g: grp_copy(ssm_hbm, ssm_buf, sem_ssm, g, False)
        def o_copy(n):
            off = pl.multiple_of(n * NC, NC)
            return pltpu.make_async_copy(out_buf.at[:, pl.ds(off, NC)], o_hbm.at[0, :, pl.ds(off, NC)], sem_o.at[n])

        q_copy(0).start(); k_copy(0).start(); v_copy(0).start()
        def early(i):
            if i == 0:
                q_copy(2).start(); w1p_copy(1).start()
            elif i == 1:
                q_copy(3).start(); w1p_copy(2).start()
            elif i == 2:
                w1p_copy(3).start()
                k_copy(1).start(); v_copy(1).start(); ssm_copy(0).start()
                w1_copy(1).start()
            elif i == 3:
                w1_copy(2).start()
                ssm_copy(1).start(); k_copy(2).start(); v_copy(2).start(); ssm_copy(2).start()

        rows = jnp.concatenate([shift_ref[...].astype(f32), dd_ref[...].astype(f32).reshape(1, D), jnp.zeros((3, D), f32)], axis=0)
        colT = jnp.concatenate([rows, jnp.zeros((120, D), f32)], axis=0).T
        for j in range(5):
            col_ref[j] = jnp.broadcast_to(colT[:, j:j + 1], (D, P))
        zero_ref[0] = 0

        def compute_kv(r0, CG=CG):
            kk = k_buf[pl.ds(r0, CG), :]
            kpad = jnp.concatenate([jnp.zeros((CG, P), bf16), kk], axis=1)
            ks = None
            for j in range(4):
                w = jnp.concatenate([col_ref[j, pl.ds(r0, CG), :]] * (S // P), axis=1)
                kj = kk if j == 0 else kpad[:, P - j:P - j + S]
                t = kj.astype(f32) * w
                ks = t if ks is None else ks + t
            kvT[pl.ds(r0, CG), :] = (ks * v_buf[pl.ds(r0, CG), :].astype(f32)).astype(bf16)

        def ln_chunk(i):
            for t in range(QC // LNC):
                off = pl.multiple_of(i * QC + t * LNC, LNC)
                xt = xT[:, pl.ds(off, LNC)].astype(f32)
                xn = ln0(xt).astype(bf16)
                xnT[:, pl.ds(off, LNC)] = xn
                hT[:, pl.ds(off, LNC)] = ln0(xn.astype(f32)).astype(bf16)
        assert NQ == 4
        with scope('ln0'):
            q_copy(0).wait()
            q_copy(1).start(); w1p_copy(0).start()
            ln_chunk(0)
            pre_ref[0] = jnp.zeros((D, FC), f32)
        def cbody(c, carry):
            for i in range(4):
                pl.when(c == i)(functools.partial(early, i))
            @pl.when(c < NQ - 1)
            def _():
                q_copy(c + 1).wait()
            w1p_copy(c).wait()
            off = pl.multiple_of(c * QC, QC)
            part = jnp.dot(hT[:, pl.ds(off, QC)], w1_buf[pl.ds(off, QC), pl.ds(0, FC)], preferred_element_type=f32)
            ln_chunk(jnp.minimum(c + 1, NQ - 1))
            compute_kv(pl.multiple_of(c * (CG // NQ), CG // NQ), CG // NQ)
            pre_ref[0] += part
            return carry
        with scope('s0wait'):
            k_copy(0).wait(); v_copy(0).wait()
        with scope('cloop'):
            jax.lax.fori_loop(0, NQ, cbody, 0)

        lane1 = jax.lax.broadcasted_iota(jnp.int32, (1, P), 1)
        sgn = jnp.where(lane1 % 2 == 0, 1.0, -1.0).astype(f32)

        XO, KO, ZO = 0, A * CG, 2 * A * CG
        def c3(zdyn):
            for g0 in range(0, CG, RG):
                ldx = lambda a, h: wk_ref[pl.ds(XO + a * CG + g0, RG), h * P:(h + 1) * P]
                ldk = lambda a, h: wk_ref[pl.ds(KO + a * CG + g0, RG), h * P:(h + 1) * P]
                for m in range(A - 1, 0, -1):
                    kr = ldk(m, 0) - sgn * ldk(m - 1, 1)
                    ki = ldk(m, 1) + sgn * ldk(m - 1, 0)
                    wk_ref[pl.ds(KO + m * CG + g0, RG), 0:P] = kr
                    wk_ref[pl.ds(KO + m * CG + g0, RG), P:2 * P] = ki
                for a0 in range(0, A, AG):
                    zr = [None] * AG; zi = [None] * AG
                    xw = {}
                    for m in range(a0 + AG):
                        kr = ldk(m, 0); ki = ldk(m, 1)
                        for t in range(AG):
                            a = a0 + t
                            if m > a: continue
                            b = a - m
                            if b not in xw:
                                xw[b] = (ldx(b, 0), ldx(b, 1))
                            xr, xi = xw[b]
                            tr = kr * xr - ki * xi
                            ti = kr * xi + ki * xr
                            zr[t] = tr if zr[t] is None else zr[t] + tr
                            zi[t] = ti if zi[t] is None else zi[t] + ti
                    for t in range(AG):
                        a = a0 + t
                        zrow = ZO + (a * CG + g0) // 2
                        if alias:
                            zrow = pl.multiple_of(zdyn + zrow, 8)
                        wk_ref[pl.ds(zrow, RG // 2), 0:P] = pltpu.bitcast(zr[t].astype(bf16), f32)
                        wk_ref[pl.ds(zrow, RG // 2), P:2 * P] = pltpu.bitcast(zi[t].astype(bf16), f32)

        def conv_fwd(r0):
            lx = jnp.concatenate([kvT[pl.ds(r0, CG), a * P:(a + 1) * P] for a in range(A)], axis=0)
            lk = jnp.concatenate([ssm_buf[pl.ds(r0, CG), a * P:(a + 1) * P] for a in range(A)], axis=0)
            wk_ref[pl.ds(XO, A * CG), :] = jnp.dot(lx, ft_ref[...], preferred_element_type=f32)
            wk_ref[pl.ds(KO, A * CG), :] = jnp.dot(lk, ft_ref[...], preferred_element_type=f32)
        def conv_inv(r0):
            yb = jnp.dot(pltpu.bitcast(wk_ref[pl.ds(ZO, A * CG // 2), :], bf16), g_ref[...], preferred_element_type=f32)
            for a in range(A):
                y_ref[pl.ds(r0, CG), a * P:(a + 1) * P] = yb[a * CG:(a + 1) * CG, :]
        def bias1(off):
            return b1_ref[pl.ds(off, FC)].astype(f32).reshape(1, FC)

        def act(j, slot):
            off = pl.multiple_of(j * FC, FC)
            u_ref[:, pl.ds(off, FC)] = gelu(pre_ref[slot] + bias1(off)).astype(bf16)

        def bodyA(j, c):
            off = pl.multiple_of(j * FC, FC)
            r0 = pl.multiple_of((j - 1) * CG, CG)
            @pl.when(j + 2 < NJ)
            def _():
                w1_copy(j + 2).start()
                k_copy(j + 2).start(); v_copy(j + 2).start(); ssm_copy(j + 2).start()
            @pl.when(j >= NJ - W2E)
            def _():
                w2_copy(j - (NJ - W2E), 0).start(); w2_copy(j - (NJ - W2E), 1).start()
            k_copy(j).wait(); v_copy(j).wait()
            w1_copy(j).wait()
            ssm_copy(j - 1).wait()
            slot = j % 2
            conv_fwd(r0)
            u = jnp.dot(hT[...], w1_buf[:, pl.ds(off, FC)], preferred_element_type=f32)
            c3(jnp.minimum(j, 0))
            act(j - 1, 1 - slot)
            conv_inv(r0)
            compute_kv(pl.multiple_of(j * CG, CG))
            pre_ref[slot] = u
            return c
        with scope('phaseA'):
            jax.lax.fori_loop(1, NJ, bodyA, 0)

        def epilogue(n, slot):
            off = pl.multiple_of(n * NC, NC)
            yy = acc_ref[slot] + b2_ref[pl.ds(off, NC)].astype(f32).reshape(1, NC)
            g = yy * jax.nn.sigmoid(yy)
            dc = jnp.concatenate([col_ref[4]] * (NC // P), axis=1)
            yv = y_ref[:, pl.ds(off, NC)] + kvT[:, pl.ds(off, NC)].astype(f32) * dc
            o = xT[:, pl.ds(off, NC)].astype(f32) + xnT[:, pl.ds(off, NC)].astype(f32) * yv * g
            out_buf[:, pl.ds(off, NC)] = o.astype(bf16)
        def mm2(off):
            return (jnp.dot(u_ref[:, 0:KH], w2a_buf[:, pl.ds(off, NC)], preferred_element_type=f32)
                    + jnp.dot(u_ref[:, KH:], w2b_buf[:, pl.ds(off, NC)], preferred_element_type=f32))

        with scope('B0'):
            w2_copy(W2E, 0).start(); w2_copy(W2E, 1).start()
            ssm_copy(NG - 1).wait()
            w2_copy(0, 0).wait(); w2_copy(0, 1).wait()
            rl = (NG - 1) * CG
            conv_fwd(rl)
            KL = F - FC
            part = (jnp.dot(u_ref[:, 0:KH], w2a_buf[:, 0:NC], preferred_element_type=f32)
                    + jnp.dot(u_ref[:, KH:KL], w2b_buf[0:KL - KH, 0:NC], preferred_element_type=f32))
            c3(zero_ref[0])
            act(NJ - 1, (NJ - 1) % 2)
            part = part + jnp.dot(u_ref[:, KL:], w2b_buf[KL - KH:, 0:NC], preferred_element_type=f32)
            conv_inv(rl)
            acc_ref[0] = part

        def bodyB(n, c):
            off = pl.multiple_of(n * NC, NC)
            @pl.when(n + W2E < NN)
            def _():
                w2_copy(n + W2E, 0).start(); w2_copy(n + W2E, 1).start()
            @pl.when(n >= 2)
            def _():
                o_copy(n - 2).start()
            w2_copy(n, 0).wait(); w2_copy(n, 1).wait()
            slot = n % 2
            epilogue(n - 1, 1 - slot)
            acc_ref[slot] = mm2(off)
            return c
        with scope('phaseB'):
            jax.lax.fori_loop(1, NN, bodyB, 0)
        with scope('tail'):
            o_copy(NN - 2).start()
            epilogue(NN - 1, (NN - 1) % 2)
            o_copy(NN - 1).start()
            for n in range(NN):
                o_copy(n).wait()

    def fn(A_q, A_k, A_v, A_shift_k, A_ssm_k, A_ssm_D, B_x, B_w1, B_b1, B_w2, B_b2):
        any_spec = pl.BlockSpec(memory_space=pltpu.HBM)
        vm = pl.BlockSpec(memory_space=pltpu.VMEM)
        outT = pl.pallas_call(
            kernel,
            out_shape=jax.ShapeDtypeStruct((1, D, S), bf16),
            in_specs=[any_spec, any_spec, any_spec, vm, any_spec, vm, any_spec, vm, any_spec, vm, vm, vm],
            out_specs=any_spec,
            scratch_shapes=[
                pltpu.VMEM((D, S), bf16), pltpu.VMEM((D, S), bf16), pltpu.VMEM((D, S), bf16), pltpu.VMEM((D, S), bf16),
                pltpu.VMEM((S, F), bf16), pltpu.VMEM((F // 2, S), bf16), pltpu.VMEM((F // 2, S), bf16),
                pltpu.VMEM((D, S), bf16), pltpu.VMEM((D, S), bf16), pltpu.VMEM((D, S), bf16),
                pltpu.VMEM((D, S), f32), pltpu.VMEM((D, F), bf16), pltpu.VMEM((D, S), bf16),
                pltpu.VMEM((2 * A * CG + A * CG // 2, 2 * P), f32), pltpu.VMEM((2, D, FC), f32), pltpu.SMEM((1,), jnp.int32),
                pltpu.VMEM((5, D, P), f32), pltpu.VMEM((2, D, NC), f32),
                pltpu.SemaphoreType.DMA((NQ,)), pltpu.SemaphoreType.DMA((NG,)), pltpu.SemaphoreType.DMA((NG,)), pltpu.SemaphoreType.DMA((NG,)),
                pltpu.SemaphoreType.DMA((NJ,)), pltpu.SemaphoreType.DMA((NQ,)), pltpu.SemaphoreType.DMA((2 * NN,)), pltpu.SemaphoreType.DMA((NN,)),
            ],
            compiler_params=pltpu.CompilerParams(vmem_limit_bytes=110 * 1024 * 1024, flags=flags),
        )(A_q.transpose(0, 2, 1), A_k.transpose(0, 2, 1), A_v.transpose(0, 2, 1), A_shift_k.T, A_ssm_k,
          A_ssm_D, B_w1, B_b1, B_w2, B_b2, FT_NP, G_NP)
        return outT.transpose(0, 2, 1)
    return fn


_KERNEL_FN = make()


@jax.jit
def pallas_recurrent_scan__ssm_conv_h3__mixer_token_mlp__prompt_kernel(
    A_q: jax.Array,
    A_k: jax.Array,
    A_v: jax.Array,
    A_shift_k: jax.Array,
    A_ssm_k: jax.Array,
    A_ssm_D: jax.Array,
    B_x: jax.Array,
    B_w1: jax.Array,
    B_b1: jax.Array,
    B_w2: jax.Array,
    B_b2: jax.Array,
):
    return _KERNEL_FN(A_q, A_k, A_v, A_shift_k, A_ssm_k, A_ssm_D, B_x, B_w1, B_b1, B_w2, B_b2)
```

```python
import functools
import numpy as np
import jax, jax.numpy as jnp
from jax.experimental import pallas as pl
from jax.experimental.pallas import tpu as pltpu

S, D, F = 2048, 576, 4608
P = 128; A = S // P
f32, bf16 = jnp.float32, jnp.bfloat16

def _dft_consts():
    r = np.arange(P, dtype=np.float64)[:, None]
    f = np.arange(P, dtype=np.float64)[None, :]
    th = np.pi * (2 * f + 1) / (2 * P)
    Ft = np.concatenate([np.cos(th * r), -np.sin(th * r)], axis=1)
    G = Ft.T / P
    return Ft.astype(jnp.bfloat16), np.ascontiguousarray(G).astype(jnp.bfloat16)
FT_NP, G_NP = _dft_consts()

def gelu(x):
    c = 0.7978845608028654
    return 0.5 * x * (1.0 + jnp.tanh(c * (x + 0.044715 * x * x * x)))

def colsum(x):
    return jnp.sum(x, axis=0, keepdims=True)

def ln0(x):
    m = colsum(x) * (1.0 / D)
    xc = x - m
    v = colsum(xc * xc) * (1.0 / D)
    return xc * jax.lax.rsqrt(v + 1e-5)

def make(FC=512, NC=256, CG=64, QC=512, LNC=256, RG=16, AG=1, scopes=False, conv=True, KB=1, W2E=2, flags=None, alias=True, late=2, sched=6, unroll_c=True, nobc=True, vmem=110):
    NJ = F // FC; NN = S // NC; NQ = S // QC; NG = D // CG
    assert NG == NJ
    import contextlib
    def scope(n):
        return jax.named_scope(n) if scopes else contextlib.nullcontext()

    def kernel(q_hbm, k_hbm, v_hbm, shift_ref, ssm_hbm, dd_ref, w1_hbm, b1_ref, w2_hbm, b2_ref,
               ft_ref, g_ref, o_hbm,
               xT, k_buf, v_buf, ssm_buf, w1_buf, w2a_buf, w2b_buf,
               xnT, hT, kvT, y_ref, u_ref, out_buf, wk_ref, pre_ref, zero_ref, col_ref, acc_ref,
               sem_q, sem_k, sem_v, sem_ssm, sem_w1, sem_w1p, sem_w2, sem_o):
        u32 = jnp.uint32
        q32, k32, v32, o32 = (r.bitcast(u32) for r in (q_hbm, k_hbm, v_hbm, o_hbm))
        ssm32, w132, w232 = (r.bitcast(u32) for r in (ssm_hbm, w1_hbm, w2_hbm))
        def ldp(ref, r0, nr, c0, nc):
            r = r0 // 2 if isinstance(r0, int) else pl.multiple_of(r0 // 2, 8)
            return pltpu.bitcast(ref[pl.ds(r, nr // 2), pl.ds(c0, nc)], bf16)
        def stp(ref, r0, nr, c0, nc, val):
            r = r0 // 2 if isinstance(r0, int) else pl.multiple_of(r0 // 2, 8)
            ref[pl.ds(r, nr // 2), pl.ds(c0, nc)] = pltpu.bitcast(val, jnp.uint32)
        def q_copy(i):
            off = pl.multiple_of(i * QC, QC)
            return pltpu.make_async_copy(q32.at[0, :, pl.ds(off, QC)], xT.at[:, pl.ds(off, QC)], sem_q.at[i])
        def w1_copy(j):
            off = pl.multiple_of(j * FC, FC)
            return pltpu.make_async_copy(w132.at[:, pl.ds(off, FC)], w1_buf.at[:, pl.ds(off, FC)], sem_w1.at[j])
        def w1p_copy(c):
            off = pl.multiple_of(c * (QC // 2), QC // 2)
            return pltpu.make_async_copy(w132.at[pl.ds(off, QC // 2), pl.ds(0, FC)], w1_buf.at[pl.ds(off, QC // 2), pl.ds(0, FC)], sem_w1p.at[c])
        KH = F // 2
        def w2_copy(n, h):
            off = pl.multiple_of(n * NC, NC)
            return pltpu.make_async_copy(w232.at[pl.ds(h * (KH // 2), KH // 2), pl.ds(off, NC)], (w2a_buf, w2b_buf)[h].at[:, pl.ds(off, NC)], sem_w2.at[2 * n + h])
        def grp_copy(hbm, buf, sem, g, three_d):
            off = pl.multiple_of(g * (CG // 2), CG // 2)
            src = hbm.at[0, pl.ds(off, CG // 2), :] if three_d else hbm.at[pl.ds(off, CG // 2), :]
            return pltpu.make_async_copy(src, buf.at[pl.ds(off, CG // 2), :], sem.at[g])
        k_copy = lambda g: grp_copy(k32, k_buf, sem_k, g, True)
        v_copy = lambda g: grp_copy(v32, v_buf, sem_v, g, True)
        ssm_copy = lambda g: grp_copy(ssm32, ssm_buf, sem_ssm, g, False)
        def o_copy(n):
            off = pl.multiple_of(n * NC, NC)
            return pltpu.make_async_copy(out_buf.at[:, pl.ds(off, NC)], o32.at[0, :, pl.ds(off, NC)], sem_o.at[n])

        def cp(name):
            kind, i = name[0], int(name[1:])
            return {'q': q_copy, 'p': w1p_copy, 'k': k_copy, 'v': v_copy, 's': ssm_copy, 'w': w1_copy}[kind](i)
        SCH = {
            0: ("q0 k0 v0", "q1 p0", ["q2 p1", "q3 p2", "p3 k1 v1 s0 w1", "w2 s1 k2 v2 s2"]),
            1: ("q0 k0 v0 q1 p0", "", ["q2 p1", "q3 p2", "p3 k1 v1 s0 w1", "w2 s1 k2 v2 s2"]),
            2: ("q0 q1 p0", "k0 v0", ["q2 p1", "q3 p2", "p3 w1 k1 v1 s0", "w2 s1 k2 v2 s2"]),
            3: ("q0 k0 v0 q1 p0", "q2 p1", ["q3 p2", "p3 w1", "k1 v1 s0", "w2 s1 k2 v2 s2"]),
            4: ("q0 k0 v0 q1 p0", "q2", ["p1 q3", "p2 p3 s0", "w1 k1 v1", "w2 s1 k2 v2 s2"]),
            5: ("q0 k0 v0", "q1 p0 q2", ["p1 q3", "p2 p3 s0 k1 v1", "w1", "w2 s1 k2 v2 s2"]),
            6: ("q0 q1 k0 v0 p0", "q2 p1", ["q3 p2 s0", "p3 k1 v1", "w1", "w2 s1 k2 v2 s2"]),
        }[sched]
        def issue(names):
            for nm in names.split():
                cp(nm).start()
        issue(SCH[0])
        def early(i):
            issue(SCH[2][i])

        rows = jnp.concatenate([shift_ref[...].astype(f32), dd_ref[...].astype(f32).reshape(1, D), jnp.zeros((3, D), f32)], axis=0)
        colT = jnp.concatenate([rows, jnp.zeros((120, D), f32)], axis=0).T
        for j in range(5):
            col_ref[j] = jnp.broadcast_to(colT[:, j:j + 1], (D, P))
        zero_ref[0] = 0

        def compute_kv(r0, CG=CG):
            kk = ldp(k_buf, r0, CG, 0, S)
            kpad = jnp.concatenate([jnp.zeros((CG, P), bf16), kk], axis=1)
            ks = None
            for j in range(4):
                w = jnp.concatenate([col_ref[j, pl.ds(r0, CG), :]] * (S // P), axis=1)
                kj = kk if j == 0 else kpad[:, P - j:P - j + S]
                t = kj.astype(f32) * w
                ks = t if ks is None else ks + t
            stp(kvT, r0, CG, 0, S, (ks * ldp(v_buf, r0, CG, 0, S).astype(f32)).astype(bf16))

        def ln_chunk(i):
            for t in range(QC // LNC):
                off = i * QC + t * LNC if isinstance(i, int) else pl.multiple_of(i * QC + t * LNC, LNC)
                xt = ldp(xT, 0, D, off, LNC).astype(f32)
                xn = ln0(xt).astype(bf16)
                stp(xnT, 0, D, off, LNC, xn)
                stp(hT, 0, D, off, LNC, ln0(xn.astype(f32)).astype(bf16))
        assert NQ == 4
        with scope('ln0'):
            q_copy(0).wait()
            issue(SCH[1])
            ln_chunk(0)
            if not unroll_c:
                pre_ref[0] = jnp.zeros((D, FC), f32)
        def cslice(c, last_ln):
            off = c * QC if isinstance(c, int) else pl.multiple_of(c * QC, QC)
            part = jnp.dot(ldp(hT, 0, D, off, QC), ldp(w1_buf, off, QC, 0, FC), preferred_element_type=f32)
            if isinstance(c, int):
                if c + 1 < NQ:
                    ln_chunk(c + 1)
                compute_kv(c * (CG // NQ), CG // NQ)
            else:
                ln_chunk(jnp.minimum(c + 1, NQ - 1))
                compute_kv(pl.multiple_of(c * (CG // NQ), CG // NQ), CG // NQ)
            if isinstance(c, int) and c == 0:
                pre_ref[0] = part
            else:
                pre_ref[0] += part
        def cbody(c, carry):
            for i in range(4):
                pl.when(c == i)(functools.partial(early, i))
            if unroll_c:
                for i in range(NQ):
                    @pl.when(c == i)
                    def _(i=i):
                        if i < NQ - 1:
                            q_copy(i + 1).wait()
                        w1p_copy(i).wait()
                        cslice(i, None)
            else:
                @pl.when(c < NQ - 1)
                def _():
                    q_copy(c + 1).wait()
                w1p_copy(c).wait()
                cslice(c, None)
            return carry
        with scope('s0wait'):
            k_copy(0).wait(); v_copy(0).wait()
        with scope('cloop'):
            jax.lax.fori_loop(0, NQ, cbody, 0)

        lane1 = jax.lax.broadcasted_iota(jnp.int32, (1, P), 1)
        sgn = jnp.where(lane1 % 2 == 0, 1.0, -1.0).astype(f32)

        XO, KO, ZO = 0, A * CG, 2 * A * CG
        def c3(zdyn):
            for g0 in range(0, CG, RG):
                ldx = lambda a, h: wk_ref[pl.ds(XO + a * CG + g0, RG), h * P:(h + 1) * P]
                ldk = lambda a, h: wk_ref[pl.ds(KO + a * CG + g0, RG), h * P:(h + 1) * P]
                for m in range(A - 1, 0, -1):
                    kr = ldk(m, 0) - sgn * ldk(m - 1, 1)
                    ki = ldk(m, 1) + sgn * ldk(m - 1, 0)
                    wk_ref[pl.ds(KO + m * CG + g0, RG), 0:P] = kr
                    wk_ref[pl.ds(KO + m * CG + g0, RG), P:2 * P] = ki
                for a0 in range(0, A, AG):
                    zr = [None] * AG; zi = [None] * AG
                    xw = {}
                    for m in range(a0 + AG):
                        kr = ldk(m, 0); ki = ldk(m, 1)
                        for t in range(AG):
                            a = a0 + t
                            if m > a: continue
                            b = a - m
                            if b not in xw:
                                xw[b] = (ldx(b, 0), ldx(b, 1))
                            xr, xi = xw[b]
                            tr = kr * xr - ki * xi
                            ti = kr * xi + ki * xr
                            zr[t] = tr if zr[t] is None else zr[t] + tr
                            zi[t] = ti if zi[t] is None else zi[t] + ti
                    for t in range(AG):
                        a = a0 + t
                        zrow = ZO + (a * CG + g0) // 2
                        if alias:
                            zrow = pl.multiple_of(zdyn + zrow, 8)
                        wk_ref[pl.ds(zrow, RG // 2), 0:P] = pltpu.bitcast(zr[t].astype(bf16), f32)
                        wk_ref[pl.ds(zrow, RG // 2), P:2 * P] = pltpu.bitcast(zi[t].astype(bf16), f32)

        def conv_fwd(r0):
            lx = jnp.concatenate([ldp(kvT, r0, CG, a * P, P) for a in range(A)], axis=0)
            lk = jnp.concatenate([ldp(ssm_buf, r0, CG, a * P, P) for a in range(A)], axis=0)
            wk_ref[pl.ds(XO, A * CG), :] = jnp.dot(lx, ft_ref[...], preferred_element_type=f32)
            wk_ref[pl.ds(KO, A * CG), :] = jnp.dot(lk, ft_ref[...], preferred_element_type=f32)
        def conv_inv(r0):
            yb = jnp.dot(pltpu.bitcast(wk_ref[pl.ds(ZO, A * CG // 2), :], bf16), g_ref[...], preferred_element_type=f32)
            for a in range(A):
                y_ref[pl.ds(r0, CG), a * P:(a + 1) * P] = yb[a * CG:(a + 1) * CG, :]
        def bias1(off):
            return b1_ref[pl.ds(off, FC)].astype(f32).reshape(1, FC)

        def act(j, slot):
            off = pl.multiple_of(j * FC, FC)
            stp(u_ref, 0, D, off, FC, gelu(pre_ref[slot] + bias1(off)).astype(bf16))

        def bodyA(j, c):
            off = pl.multiple_of(j * FC, FC)
            r0 = pl.multiple_of((j - 1) * CG, CG)
            @pl.when(j + 2 < NJ)
            def _():
                w1_copy(j + 2).start()
                k_copy(j + 2).start(); v_copy(j + 2).start(); ssm_copy(j + 2).start()
            @pl.when(j >= NJ - W2E)
            def _():
                w2_copy(j - (NJ - W2E), 0).start(); w2_copy(j - (NJ - W2E), 1).start()
            k_copy(j).wait(); v_copy(j).wait()
            w1_copy(j).wait()
            ssm_copy(j - 1).wait()
            slot = j % 2
            conv_fwd(r0)
            u = jnp.dot(ldp(hT, 0, D, 0, S), ldp(w1_buf, 0, S, off, FC), preferred_element_type=f32)
            c3(jnp.minimum(j, 0))
            act(j - 1, 1 - slot)
            conv_inv(r0)
            compute_kv(pl.multiple_of(j * CG, CG))
            pre_ref[slot] = u
            return c
        with scope('phaseA'):
            jax.lax.fori_loop(1, NJ, bodyA, 0)

        def epilogue(n, slot):
            off = pl.multiple_of(n * NC, NC)
            yy = acc_ref[slot] + b2_ref[pl.ds(off, NC)].astype(f32).reshape(1, NC)
            g = yy * jax.nn.sigmoid(yy)
            dc = jnp.concatenate([col_ref[4]] * (NC // P), axis=1)
            yv = y_ref[:, pl.ds(off, NC)] + ldp(kvT, 0, D, off, NC).astype(f32) * dc
            o = ldp(xT, 0, D, off, NC).astype(f32) + ldp(xnT, 0, D, off, NC).astype(f32) * yv * g
            stp(out_buf, 0, D, off, NC, o.astype(bf16))
        def mm2(off):
            return (jnp.dot(ldp(u_ref, 0, D, 0, KH), ldp(w2a_buf, 0, KH, off, NC), preferred_element_type=f32)
                    + jnp.dot(ldp(u_ref, 0, D, KH, KH), ldp(w2b_buf, 0, KH, off, NC), preferred_element_type=f32))

        with scope('B0'):
            w2_copy(W2E, 0).start(); w2_copy(W2E, 1).start()
            ssm_copy(NG - 1).wait()
            w2_copy(0, 0).wait(); w2_copy(0, 1).wait()
            rl = (NG - 1) * CG
            conv_fwd(rl)
            KL = F - FC
            part = (jnp.dot(ldp(u_ref, 0, D, 0, KH), ldp(w2a_buf, 0, KH, 0, NC), preferred_element_type=f32)
                    + jnp.dot(ldp(u_ref, 0, D, KH, KL - KH), ldp(w2b_buf, 0, KL - KH, 0, NC), preferred_element_type=f32))
            c3(zero_ref[0])
            act(NJ - 1, (NJ - 1) % 2)
            part = part + jnp.dot(ldp(u_ref, 0, D, KL, FC), ldp(w2b_buf, KL - KH, FC, 0, NC), preferred_element_type=f32)
            conv_inv(rl)
            acc_ref[0] = part

        def bodyB(n, c):
            off = pl.multiple_of(n * NC, NC)
            @pl.when(n + W2E < NN)
            def _():
                w2_copy(n + W2E, 0).start(); w2_copy(n + W2E, 1).start()
            @pl.when(n >= 2)
            def _():
                o_copy(n - 2).start()
            w2_copy(n, 0).wait(); w2_copy(n, 1).wait()
            slot = n % 2
            epilogue(n - 1, 1 - slot)
            acc_ref[slot] = mm2(off)
            return c
        with scope('phaseB'):
            jax.lax.fori_loop(1, NN, bodyB, 0)
        with scope('tail'):
            o_copy(NN - 2).start()
            epilogue(NN - 1, (NN - 1) % 2)
            o_copy(NN - 1).start()
            for n in range(NN):
                o_copy(n).wait()

    def fn(A_q, A_k, A_v, A_shift_k, A_ssm_k, A_ssm_D, B_x, B_w1, B_b1, B_w2, B_b2):
        any_spec = pl.BlockSpec(memory_space=pltpu.HBM)
        vm = pl.BlockSpec(memory_space=pltpu.VMEM)
        outT = pl.pallas_call(
            kernel,
            out_shape=jax.ShapeDtypeStruct((1, D, S), bf16),
            in_specs=[any_spec, any_spec, any_spec, vm, any_spec, vm, any_spec, vm, any_spec, vm, vm, vm],
            out_specs=any_spec,
            scratch_shapes=[
                pltpu.VMEM((D // 2, S), jnp.uint32), pltpu.VMEM((D // 2, S), jnp.uint32), pltpu.VMEM((D // 2, S), jnp.uint32), pltpu.VMEM((D // 2, S), jnp.uint32),
                pltpu.VMEM((S // 2, F), jnp.uint32), pltpu.VMEM((F // 4, S), jnp.uint32), pltpu.VMEM((F // 4, S), jnp.uint32),
                pltpu.VMEM((D // 2, S), jnp.uint32), pltpu.VMEM((D // 2, S), jnp.uint32), pltpu.VMEM((D // 2, S), jnp.uint32),
                pltpu.VMEM((D, S), f32), pltpu.VMEM((D // 2, F), jnp.uint32), pltpu.VMEM((D // 2, S), jnp.uint32),
                pltpu.VMEM((2 * A * CG + A * CG // 2, 2 * P), f32), pltpu.VMEM((2, D, FC), f32), pltpu.SMEM((1,), jnp.int32),
                pltpu.VMEM((5, D, P), f32), pltpu.VMEM((2, D, NC), f32),
                pltpu.SemaphoreType.DMA((NQ,)), pltpu.SemaphoreType.DMA((NG,)), pltpu.SemaphoreType.DMA((NG,)), pltpu.SemaphoreType.DMA((NG,)),
                pltpu.SemaphoreType.DMA((NJ,)), pltpu.SemaphoreType.DMA((NQ,)), pltpu.SemaphoreType.DMA((2 * NN,)), pltpu.SemaphoreType.DMA((NN,)),
            ],
            compiler_params=pltpu.CompilerParams(vmem_limit_bytes=vmem * 1024 * 1024, flags=flags, disable_bounds_checks=nobc),
        )(A_q.transpose(0, 2, 1), A_k.transpose(0, 2, 1), A_v.transpose(0, 2, 1), A_shift_k.T, A_ssm_k,
          A_ssm_D, B_w1, B_b1, B_w2, B_b2, FT_NP, G_NP)
        return outT.transpose(0, 2, 1)
    return fn


_KERNEL_FN = make()


@jax.jit
def pallas_recurrent_scan__ssm_conv_h3__mixer_token_mlp__prompt_kernel(
    A_q: jax.Array,
    A_k: jax.Array,
    A_v: jax.Array,
    A_shift_k: jax.Array,
    A_ssm_k: jax.Array,
    A_ssm_D: jax.Array,
    B_x: jax.Array,
    B_w1: jax.Array,
    B_b1: jax.Array,
    B_w2: jax.Array,
    B_b2: jax.Array,
):
    return _KERNEL_FN(A_q, A_k, A_v, A_shift_k, A_ssm_k, A_ssm_D, B_x, B_w1, B_b1, B_w2, B_b2)
```

```python
import functools
import numpy as np
import jax, jax.numpy as jnp
from jax.experimental import pallas as pl
from jax.experimental.pallas import tpu as pltpu

S, D, F = 2048, 576, 4608
P = 128; A = S // P
f32, bf16 = jnp.float32, jnp.bfloat16

def _dft_consts():
    r = np.arange(P, dtype=np.float64)[:, None]
    f = np.arange(P, dtype=np.float64)[None, :]
    th = np.pi * (2 * f + 1) / (2 * P)
    Ft = np.concatenate([np.cos(th * r), -np.sin(th * r)], axis=1)
    G = Ft.T / P
    return Ft.astype(jnp.bfloat16), np.ascontiguousarray(G).astype(jnp.bfloat16)
FT_NP, G_NP = _dft_consts()

def gelu(x):
    c = 0.7978845608028654
    return 0.5 * x * (1.0 + jnp.tanh(c * (x + 0.044715 * x * x * x)))

def colsum(x):
    return jnp.sum(x, axis=0, keepdims=True)

def ln0(x):
    m = colsum(x) * (1.0 / D)
    xc = x - m
    v = colsum(xc * xc) * (1.0 / D)
    return xc * jax.lax.rsqrt(v + 1e-5)

def make(FC=512, NC=256, CG=64, QC=512, LNC=256, RG=16, AG=1, scopes=False, conv=True, KB=1, W2E=2, flags=None, alias=True, sched=5, nobc=True, vmem=110, colpos=0, cv=1, LNI=128, split0=False):
    NJ = F // FC; NN = S // NC; NQ = S // QC; NG = D // CG
    assert NG == NJ
    import contextlib
    def scope(n):
        return jax.named_scope(n) if scopes else contextlib.nullcontext()

    def kernel(q_hbm, k_hbm, v_hbm, shift_ref, ssm_hbm, dd_ref, w1_hbm, b1_ref, w2_hbm, b2_ref,
               ft_ref, g_ref, o_hbm,
               xT, k_buf, v_buf, ssm_buf, w1_buf, w2a_buf, w2b_buf,
               xnT, hT, kvT, y_ref, u_ref, out_buf, wk_ref, pre_ref, zero_ref, col_ref, acc_ref,
               sem_q, sem_k, sem_v, sem_ssm, sem_w1, sem_w1p, sem_w2, sem_o):
        u32 = jnp.uint32
        q32, k32, v32, o32 = (r.bitcast(u32) for r in (q_hbm, k_hbm, v_hbm, o_hbm))
        ssm32, w132, w232 = (r.bitcast(u32) for r in (ssm_hbm, w1_hbm, w2_hbm))
        def ldp(ref, r0, nr, c0, nc):
            r = r0 // 2 if isinstance(r0, int) else pl.multiple_of(r0 // 2, 8)
            return pltpu.bitcast(ref[pl.ds(r, nr // 2), pl.ds(c0, nc)], bf16)
        def stp(ref, r0, nr, c0, nc, val):
            r = r0 // 2 if isinstance(r0, int) else pl.multiple_of(r0 // 2, 8)
            ref[pl.ds(r, nr // 2), pl.ds(c0, nc)] = pltpu.bitcast(val, jnp.uint32)
        def q_copy(i):
            off = pl.multiple_of(i * QC, QC)
            return pltpu.make_async_copy(q32.at[0, :, pl.ds(off, QC)], xT.at[:, pl.ds(off, QC)], sem_q.at[i])
        def w1_copy(j):
            off = pl.multiple_of(j * FC, FC)
            return pltpu.make_async_copy(w132.at[:, pl.ds(off, FC)], w1_buf.at[:, pl.ds(off, FC)], sem_w1.at[j])
        def w1p_copy(c):
            off = pl.multiple_of(c * (QC // 2), QC // 2)
            return pltpu.make_async_copy(w132.at[pl.ds(off, QC // 2), pl.ds(0, 2 * FC)], w1_buf.at[pl.ds(off, QC // 2), pl.ds(0, 2 * FC)], sem_w1p.at[c])
        KH = F // 2
        def w2_copy(n, h):
            off = pl.multiple_of(n * NC, NC)
            return pltpu.make_async_copy(w232.at[pl.ds(h * (KH // 2), KH // 2), pl.ds(off, NC)], (w2a_buf, w2b_buf)[h].at[:, pl.ds(off, NC)], sem_w2.at[2 * n + h])
        def grp_copy(hbm, buf, sem, g, three_d):
            off = pl.multiple_of(g * (CG // 2), CG // 2)
            src = hbm.at[0, pl.ds(off, CG // 2), :] if three_d else hbm.at[pl.ds(off, CG // 2), :]
            return pltpu.make_async_copy(src, buf.at[pl.ds(off, CG // 2), :], sem.at[g])
        k_copy = lambda g: grp_copy(k32, k_buf, sem_k, g, True)
        v_copy = lambda g: grp_copy(v32, v_buf, sem_v, g, True)
        ssm_copy = lambda g: grp_copy(ssm32, ssm_buf, sem_ssm, g, False)
        def o_copy(n):
            off = pl.multiple_of(n * NC, NC)
            return pltpu.make_async_copy(out_buf.at[:, pl.ds(off, NC)], o32.at[0, :, pl.ds(off, NC)], sem_o.at[n])

        def w1h_copy(h):
            return pltpu.make_async_copy(w132.at[pl.ds(0, QC // 2), pl.ds(h * FC, FC)], w1_buf.at[pl.ds(0, QC // 2), pl.ds(h * FC, FC)], sem_w1.at[h])
        def cp(name):
            if name[0] == 'h':
                return w1h_copy(int(name[1:]))
            kind, i = name[0], int(name[1:])
            return {'q': q_copy, 'p': w1p_copy, 'k': k_copy, 'v': v_copy, 's': ssm_copy, 'w': w1_copy}[kind](i)
        SCH = {
            0: ("q0 q1 p0", "", ["q2 p1 k0 v0", "q3 p2 s0", "p3 k1 v1", "w2 s1 k2 v2 w3 s2 k3 v3 s3"]),
            1: ("q0", "q1 p0", ["q2 p1 k0 v0", "q3 p2 s0", "p3 k1 v1", "w2 s1 k2 v2 w3 s2 k3 v3 s3"]),
            2: ("q0 q1 p0", "q2 p1", ["k0 v0 q3 p2", "s0 p3 k1 v1", "w2 s1 k2 v2", "w3 s2 k3 v3 s3"]),
            3: ("q0 q1", "p0 q2", ["p1 k0 v0 q3", "p2 s0 p3", "k1 v1 w2 s1", "k2 v2 w3 s2 k3 v3 s3"]),
            6: ("q0 h0", "q1 h1", ["q2 p1 k0 v0", "q3 p2 k1 v1", "p3 s0", "w2 s1 k2 v2 w3 s2 k3 v3 s3"]),
            7: ("q0 h0 q1", "h1", ["q2 p1 k0 v0", "q3 p2 k1 v1", "p3 s0", "w2 s1 k2 v2 w3 s2 k3 v3 s3"]),
            8: ("q0", "h0 q1 h1", ["q2 p1 k0 v0", "q3 p2 k1 v1", "p3 s0", "w2 s1 k2 v2 w3 s2 k3 v3 s3"]),
            5: ("q0 q1 p0", "", ["q2 p1 k0 v0", "q3 p2 k1 v1", "p3 s0", "w2 s1 k2 v2 w3 s2 k3 v3 s3"]),
            4: ("q0", "q1 p0 q2", ["p1 k0 v0", "q3 p2 s0 k1 v1", "p3 w2 s1", "k2 v2 w3 s2 k3 v3 s3"]),
        }[sched]
        def issue(names):
            for nm in names.split():
                cp(nm).start()
        issue(SCH[0])
        def early(i):
            issue(SCH[2][i])

        def col_prep():
            rows = jnp.concatenate([shift_ref[...].astype(f32), dd_ref[...].astype(f32).reshape(1, D), jnp.zeros((3, D), f32)], axis=0)
            colT = jnp.concatenate([rows, jnp.zeros((120, D), f32)], axis=0).T
            for j in range(5):
                col_ref[j] = jnp.broadcast_to(colT[:, j:j + 1], (D, P))
        zero_ref[0] = 0
        if colpos == 0:
            with scope('col'):
                col_prep()

        def compute_kv(r0, CG=CG):
            kk = ldp(k_buf, r0, CG, 0, S)
            kpad = jnp.concatenate([jnp.zeros((CG, P), bf16), kk], axis=1)
            ks = None
            for j in range(4):
                w = jnp.concatenate([col_ref[j, pl.ds(r0, CG), :]] * (S // P), axis=1)
                kj = kk if j == 0 else kpad[:, P - j:P - j + S]
                t = kj.astype(f32) * w
                ks = t if ks is None else ks + t
            stp(kvT, r0, CG, 0, S, (ks * ldp(v_buf, r0, CG, 0, S).astype(f32)).astype(bf16))

        lane1 = jax.lax.broadcasted_iota(jnp.int32, (1, P), 1)
        sgn = jnp.where(lane1 % 2 == 0, 1.0, -1.0).astype(f32)

        XO, KO, ZO = 0, A * CG, 2 * A * CG
        def c3(zdyn, glo=0, ghi=CG):
            for g0 in range(glo, ghi, RG):
                ldx = lambda a, h: wk_ref[pl.ds(XO + a * CG + g0, RG), h * P:(h + 1) * P]
                ldk = lambda a, h: wk_ref[pl.ds(KO + a * CG + g0, RG), h * P:(h + 1) * P]
                for m in range(A - 1, 0, -1):
                    kr = ldk(m, 0) - sgn * ldk(m - 1, 1)
                    ki = ldk(m, 1) + sgn * ldk(m - 1, 0)
                    wk_ref[pl.ds(KO + m * CG + g0, RG), 0:P] = kr
                    wk_ref[pl.ds(KO + m * CG + g0, RG), P:2 * P] = ki
                for a0 in range(0, A, AG):
                    zr = [None] * AG; zi = [None] * AG
                    xw = {}
                    for m in range(a0 + AG):
                        kr = ldk(m, 0); ki = ldk(m, 1)
                        for t in range(AG):
                            a = a0 + t
                            if m > a: continue
                            b = a - m
                            if b not in xw:
                                xw[b] = (ldx(b, 0), ldx(b, 1))
                            xr, xi = xw[b]
                            tr = kr * xr - ki * xi
                            ti = kr * xi + ki * xr
                            zr[t] = tr if zr[t] is None else zr[t] + tr
                            zi[t] = ti if zi[t] is None else zi[t] + ti
                    for t in range(AG):
                        a = a0 + t
                        zrow = ZO + (a * CG + g0) // 2
                        if alias:
                            zrow = pl.multiple_of(zdyn + zrow, 8)
                        wk_ref[pl.ds(zrow, RG // 2), 0:P] = pltpu.bitcast(zr[t].astype(bf16), f32)
                        wk_ref[pl.ds(zrow, RG // 2), P:2 * P] = pltpu.bitcast(zi[t].astype(bf16), f32)

        def conv_fwd(r0):
            lx = jnp.concatenate([ldp(kvT, r0, CG, a * P, P) for a in range(A)], axis=0)
            lk = jnp.concatenate([ldp(ssm_buf, r0, CG, a * P, P) for a in range(A)], axis=0)
            wk_ref[pl.ds(XO, A * CG), :] = jnp.dot(lx, ft_ref[...], preferred_element_type=f32)
            wk_ref[pl.ds(KO, A * CG), :] = jnp.dot(lk, ft_ref[...], preferred_element_type=f32)
        def conv_inv(r0):
            yb = jnp.dot(pltpu.bitcast(wk_ref[pl.ds(ZO, A * CG // 2), :], bf16), g_ref[...], preferred_element_type=f32)
            for a in range(A):
                y_ref[pl.ds(r0, CG), a * P:(a + 1) * P] = yb[a * CG:(a + 1) * CG, :]
        def bias1(off):
            return b1_ref[pl.ds(off, FC)].astype(f32).reshape(1, FC)

        def act(j, slot):
            off = pl.multiple_of(j * FC, FC)
            stp(u_ref, 0, D, off, FC, gelu(pre_ref[slot] + bias1(off)).astype(bf16))

        def ln_chunk(i, LNC=LNC):
            for t in range(QC // LNC):
                off = i * QC + t * LNC if isinstance(i, int) else pl.multiple_of(i * QC + t * LNC, LNC)
                xt = ldp(xT, 0, D, off, LNC).astype(f32)
                xn = ln0(xt).astype(bf16)
                stp(xnT, 0, D, off, LNC, xn)
                stp(hT, 0, D, off, LNC, ln0(xn.astype(f32)).astype(bf16))
        assert NQ == 4
        with scope('ln0'):
            q_copy(0).wait()
            issue(SCH[1])
            ln_chunk(0)
            if colpos == 1:
                col_prep()
        F0 = 2 * FC
        def kslice(c):
            off = c * QC
            if c < NQ - 1:
                q_copy(c + 1).wait()
            if c == 1:
                k_copy(0).wait(); v_copy(0).wait()
            if c == (2 if cv == 0 else 3):
                ssm_copy(0).wait()
            if c == (3 if cv == 0 else 2):
                k_copy(1).wait(); v_copy(1).wait()
            if c == 0 and split0:
                w1h_copy(1).wait()
                pre_ref[1] = jnp.dot(ldp(hT, 0, D, 0, QC), ldp(w1_buf, 0, QC, FC, FC), preferred_element_type=f32)
                ln_chunk(1, LNI)
                return
            w1p_copy(c).wait()
            lhs = ldp(hT, 0, D, off, QC)
            if c == (2 if cv == 0 else 3):
                conv_fwd(0)
            pab = jnp.dot(lhs, ldp(w1_buf, off, QC, 0, F0), preferred_element_type=f32)
            pa = pab[:, 0:FC]
            pb = pab[:, FC:F0]
            if c < NQ - 1:
                ln_chunk(c + 1, LNI)
            if c == 1:
                compute_kv(0)
            if c == 2 and cv == 0:
                c3(zero_ref[0], 0, CG // 2)
            if c == 2 and cv == 1:
                compute_kv(CG)
            if c == 0:
                pre_ref[0] = pa
                pre_ref[1] = pb
            elif c < NQ - 1:
                pre_ref[0] += pa
                pre_ref[1] += pb
            else:
                c3(zero_ref[0], CG // 2 if cv == 0 else 0, CG)
                if cv == 0:
                    compute_kv(CG)
                stp(u_ref, 0, D, 0, FC, gelu(pre_ref[0] + pa + bias1(0)).astype(bf16))
                pre_ref[1] += pb
                conv_inv(0)
        if split0:
            @pl.when(zero_ref[0] == 0)
            def _():
                w1h_copy(0).wait()
                pre_ref[0] = jnp.dot(ldp(hT, 0, D, 0, QC), ldp(w1_buf, 0, QC, 0, FC), preferred_element_type=f32)
        def cbody(c, carry):
            for i in range(NQ):
                pl.when(c == i)(functools.partial(early, i))
            for i in range(NQ):
                pl.when(c == i)(functools.partial(kslice, i))
            return carry
        with scope('cloop'):
            jax.lax.fori_loop(0, NQ, cbody, 0)


        def bodyA(j, c):
            off = pl.multiple_of(j * FC, FC)
            r0 = pl.multiple_of((j - 1) * CG, CG)
            @pl.when(j + 2 < NJ)
            def _():
                w1_copy(j + 2).start()
                k_copy(j + 2).start(); v_copy(j + 2).start(); ssm_copy(j + 2).start()
            @pl.when(j >= NJ - W2E)
            def _():
                w2_copy(j - (NJ - W2E), 0).start(); w2_copy(j - (NJ - W2E), 1).start()
            k_copy(j).wait(); v_copy(j).wait()
            w1_copy(j).wait()
            ssm_copy(j - 1).wait()
            slot = j % 2
            conv_fwd(r0)
            u = jnp.dot(ldp(hT, 0, D, 0, S), ldp(w1_buf, 0, S, off, FC), preferred_element_type=f32)
            c3(jnp.minimum(j, 0))
            act(j - 1, 1 - slot)
            conv_inv(r0)
            compute_kv(pl.multiple_of(j * CG, CG))
            pre_ref[slot] = u
            return c
        with scope('phaseA'):
            jax.lax.fori_loop(2, NJ, bodyA, 0)

        def epilogue(n, slot):
            off = pl.multiple_of(n * NC, NC)
            yy = acc_ref[slot] + b2_ref[pl.ds(off, NC)].astype(f32).reshape(1, NC)
            g = yy * jax.nn.sigmoid(yy)
            dc = jnp.concatenate([col_ref[4]] * (NC // P), axis=1)
            yv = y_ref[:, pl.ds(off, NC)] + ldp(kvT, 0, D, off, NC).astype(f32) * dc
            o = ldp(xT, 0, D, off, NC).astype(f32) + ldp(xnT, 0, D, off, NC).astype(f32) * yv * g
            stp(out_buf, 0, D, off, NC, o.astype(bf16))
        def mm2(off):
            return (jnp.dot(ldp(u_ref, 0, D, 0, KH), ldp(w2a_buf, 0, KH, off, NC), preferred_element_type=f32)
                    + jnp.dot(ldp(u_ref, 0, D, KH, KH), ldp(w2b_buf, 0, KH, off, NC), preferred_element_type=f32))

        with scope('B0'):
            w2_copy(W2E, 0).start(); w2_copy(W2E, 1).start()
            ssm_copy(NG - 1).wait()
            w2_copy(0, 0).wait(); w2_copy(0, 1).wait()
            rl = (NG - 1) * CG
            conv_fwd(rl)
            KL = F - FC
            part = (jnp.dot(ldp(u_ref, 0, D, 0, KH), ldp(w2a_buf, 0, KH, 0, NC), preferred_element_type=f32)
                    + jnp.dot(ldp(u_ref, 0, D, KH, KL - KH), ldp(w2b_buf, 0, KL - KH, 0, NC), preferred_element_type=f32))
            c3(zero_ref[0])
            act(NJ - 1, (NJ - 1) % 2)
            part = part + jnp.dot(ldp(u_ref, 0, D, KL, FC), ldp(w2b_buf, KL - KH, FC, 0, NC), preferred_element_type=f32)
            conv_inv(rl)
            acc_ref[0] = part

        def bodyB(n, c):
            off = pl.multiple_of(n * NC, NC)
            @pl.when(n + W2E < NN)
            def _():
                w2_copy(n + W2E, 0).start(); w2_copy(n + W2E, 1).start()
            @pl.when(n >= 2)
            def _():
                o_copy(n - 2).start()
            w2_copy(n, 0).wait(); w2_copy(n, 1).wait()
            slot = n % 2
            epilogue(n - 1, 1 - slot)
            acc_ref[slot] = mm2(off)
            return c
        with scope('phaseB'):
            jax.lax.fori_loop(1, NN, bodyB, 0)
        with scope('tail'):
            o_copy(NN - 2).start()
            epilogue(NN - 1, (NN - 1) % 2)
            o_copy(NN - 1).start()
            for n in range(NN):
                o_copy(n).wait()

    def fn(A_q, A_k, A_v, A_shift_k, A_ssm_k, A_ssm_D, B_x, B_w1, B_b1, B_w2, B_b2):
        any_spec = pl.BlockSpec(memory_space=pltpu.HBM)
        vm = pl.BlockSpec(memory_space=pltpu.VMEM)
        outT = pl.pallas_call(
            kernel,
            out_shape=jax.ShapeDtypeStruct((1, D, S), bf16),
            in_specs=[any_spec, any_spec, any_spec, vm, any_spec, vm, any_spec, vm, any_spec, vm, vm, vm],
            out_specs=any_spec,
            scratch_shapes=[
                pltpu.VMEM((D // 2, S), jnp.uint32), pltpu.VMEM((D // 2, S), jnp.uint32), pltpu.VMEM((D // 2, S), jnp.uint32), pltpu.VMEM((D // 2, S), jnp.uint32),
                pltpu.VMEM((S // 2, F), jnp.uint32), pltpu.VMEM((F // 4, S), jnp.uint32), pltpu.VMEM((F // 4, S), jnp.uint32),
                pltpu.VMEM((D // 2, S), jnp.uint32), pltpu.VMEM((D // 2, S), jnp.uint32), pltpu.VMEM((D // 2, S), jnp.uint32),
                pltpu.VMEM((D, S), f32), pltpu.VMEM((D // 2, F), jnp.uint32), pltpu.VMEM((D // 2, S), jnp.uint32),
                pltpu.VMEM((2 * A * CG + A * CG // 2, 2 * P), f32), pltpu.VMEM((2, D, FC), f32), pltpu.SMEM((1,), jnp.int32),
                pltpu.VMEM((5, D, P), f32), pltpu.VMEM((2, D, NC), f32),
                pltpu.SemaphoreType.DMA((NQ,)), pltpu.SemaphoreType.DMA((NG,)), pltpu.SemaphoreType.DMA((NG,)), pltpu.SemaphoreType.DMA((NG,)),
                pltpu.SemaphoreType.DMA((NJ,)), pltpu.SemaphoreType.DMA((NQ,)), pltpu.SemaphoreType.DMA((2 * NN,)), pltpu.SemaphoreType.DMA((NN,)),
            ],
            compiler_params=pltpu.CompilerParams(vmem_limit_bytes=vmem * 1024 * 1024, flags=flags, disable_bounds_checks=nobc),
        )(A_q.transpose(0, 2, 1), A_k.transpose(0, 2, 1), A_v.transpose(0, 2, 1), A_shift_k.T, A_ssm_k,
          A_ssm_D, B_w1, B_b1, B_w2, B_b2, FT_NP, G_NP)
        return outT.transpose(0, 2, 1)
    return fn


_KERNEL_FN = make()


@jax.jit
def pallas_recurrent_scan__ssm_conv_h3__mixer_token_mlp__prompt_kernel(
    A_q: jax.Array,
    A_k: jax.Array,
    A_v: jax.Array,
    A_shift_k: jax.Array,
    A_ssm_k: jax.Array,
    A_ssm_D: jax.Array,
    B_x: jax.Array,
    B_w1: jax.Array,
    B_b1: jax.Array,
    B_w2: jax.Array,
    B_b2: jax.Array,
):
    return _KERNEL_FN(A_q, A_k, A_v, A_shift_k, A_ssm_k, A_ssm_D, B_x, B_w1, B_b1, B_w2, B_b2)
```

```python
import functools
import numpy as np
import jax, jax.numpy as jnp
from jax.experimental import pallas as pl
from jax.experimental.pallas import tpu as pltpu

S, D, F = 2048, 576, 4608
P = 128; A = S // P
f32, bf16 = jnp.float32, jnp.bfloat16

def _dft_consts():
    r = np.arange(P, dtype=np.float64)[:, None]
    f = np.arange(P, dtype=np.float64)[None, :]
    th = np.pi * (2 * f + 1) / (2 * P)
    Ft = np.concatenate([np.cos(th * r), -np.sin(th * r)], axis=1)
    G = Ft.T / P
    return Ft.astype(jnp.bfloat16), np.ascontiguousarray(G).astype(jnp.bfloat16)
FT_NP, G_NP = _dft_consts()

def gelu(x):
    c = 0.7978845608028654
    hx = 0.5 * x
    return hx * jnp.tanh(x * (c + (c * 0.044715) * (x * x))) + hx

def silu(y):
    h = 0.5 * y
    return h * jnp.tanh(h) + h

def colsum(x):
    return jnp.sum(x, axis=0, keepdims=True)

def ln0(x):
    m = colsum(x) * (1.0 / D)
    xc = x - m
    v = colsum(xc * xc) * (1.0 / D)
    return xc * jax.lax.rsqrt(v + 1e-5)

def make(FC=512, NC=256, CG=64, QC=512, LNC=256, RG=32, AG=1, scopes=False, conv=True, KB=1, W2E=2, flags=None, alias=True, sched=5, nobc=True, vmem=110, colpos=0, cv=1, LNI=128, split0=False):
    NJ = F // FC; NN = S // NC; NQ = S // QC; NG = D // CG
    assert NG == NJ
    import contextlib
    def scope(n):
        return jax.named_scope(n) if scopes else contextlib.nullcontext()

    def kernel(q_hbm, k_hbm, v_hbm, shift_ref, ssm_hbm, dd_ref, w1_hbm, b1_ref, w2_hbm, b2_ref,
               ft_ref, g_ref, o_hbm,
               xT, k_buf, v_buf, ssm_buf, w1_buf, w2a_buf, w2b_buf,
               xnT, hT, kvT, y_ref, u_ref, out_buf, wk_ref, pre_ref, zero_ref, col_ref, acc_ref,
               sem_q, sem_k, sem_v, sem_ssm, sem_w1, sem_w1p, sem_w2, sem_o):
        u32 = jnp.uint32
        q32, k32, v32, o32 = (r.bitcast(u32) for r in (q_hbm, k_hbm, v_hbm, o_hbm))
        ssm32, w132, w232 = (r.bitcast(u32) for r in (ssm_hbm, w1_hbm, w2_hbm))
        def ldp(ref, r0, nr, c0, nc):
            r = r0 // 2 if isinstance(r0, int) else pl.multiple_of(r0 // 2, 8)
            return pltpu.bitcast(ref[pl.ds(r, nr // 2), pl.ds(c0, nc)], bf16)
        def stp(ref, r0, nr, c0, nc, val):
            r = r0 // 2 if isinstance(r0, int) else pl.multiple_of(r0 // 2, 8)
            ref[pl.ds(r, nr // 2), pl.ds(c0, nc)] = pltpu.bitcast(val, jnp.uint32)
        def q_copy(i):
            off = pl.multiple_of(i * QC, QC)
            return pltpu.make_async_copy(q32.at[0, :, pl.ds(off, QC)], xT.at[:, pl.ds(off, QC)], sem_q.at[i])
        def w1_copy(j):
            off = pl.multiple_of(j * FC, FC)
            return pltpu.make_async_copy(w132.at[:, pl.ds(off, FC)], w1_buf.at[:, pl.ds(off, FC)], sem_w1.at[j])
        def w1p_copy(c):
            off = pl.multiple_of(c * (QC // 2), QC // 2)
            return pltpu.make_async_copy(w132.at[pl.ds(off, QC // 2), pl.ds(0, 2 * FC)], w1_buf.at[pl.ds(off, QC // 2), pl.ds(0, 2 * FC)], sem_w1p.at[c])
        KH = F // 2
        def w2_copy(n, h):
            off = pl.multiple_of(n * NC, NC)
            return pltpu.make_async_copy(w232.at[pl.ds(h * (KH // 2), KH // 2), pl.ds(off, NC)], (w2a_buf, w2b_buf)[h].at[:, pl.ds(off, NC)], sem_w2.at[2 * n + h])
        def grp_copy(hbm, buf, sem, g, three_d):
            off = pl.multiple_of(g * (CG // 2), CG // 2)
            src = hbm.at[0, pl.ds(off, CG // 2), :] if three_d else hbm.at[pl.ds(off, CG // 2), :]
            return pltpu.make_async_copy(src, buf.at[pl.ds(off, CG // 2), :], sem.at[g])
        k_copy = lambda g: grp_copy(k32, k_buf, sem_k, g, True)
        v_copy = lambda g: grp_copy(v32, v_buf, sem_v, g, True)
        ssm_copy = lambda g: grp_copy(ssm32, ssm_buf, sem_ssm, g, False)
        def o_copy(n):
            off = pl.multiple_of(n * NC, NC)
            return pltpu.make_async_copy(out_buf.at[:, pl.ds(off, NC)], o32.at[0, :, pl.ds(off, NC)], sem_o.at[n])

        def w1h_copy(h):
            return pltpu.make_async_copy(w132.at[pl.ds(0, QC // 2), pl.ds(h * FC, FC)], w1_buf.at[pl.ds(0, QC // 2), pl.ds(h * FC, FC)], sem_w1.at[h])
        def cp(name):
            if name[0] == 'h':
                return w1h_copy(int(name[1:]))
            kind, i = name[0], int(name[1:])
            return {'q': q_copy, 'p': w1p_copy, 'k': k_copy, 'v': v_copy, 's': ssm_copy, 'w': w1_copy}[kind](i)
        SCH = {
            0: ("q0 q1 p0", "", ["q2 p1 k0 v0", "q3 p2 s0", "p3 k1 v1", "w2 s1 k2 v2 w3 s2 k3 v3 s3"]),
            1: ("q0", "q1 p0", ["q2 p1 k0 v0", "q3 p2 s0", "p3 k1 v1", "w2 s1 k2 v2 w3 s2 k3 v3 s3"]),
            2: ("q0 q1 p0", "q2 p1", ["k0 v0 q3 p2", "s0 p3 k1 v1", "w2 s1 k2 v2", "w3 s2 k3 v3 s3"]),
            3: ("q0 q1", "p0 q2", ["p1 k0 v0 q3", "p2 s0 p3", "k1 v1 w2 s1", "k2 v2 w3 s2 k3 v3 s3"]),
            6: ("q0 h0", "q1 h1", ["q2 p1 k0 v0", "q3 p2 k1 v1", "p3 s0", "w2 s1 k2 v2 w3 s2 k3 v3 s3"]),
            7: ("q0 h0 q1", "h1", ["q2 p1 k0 v0", "q3 p2 k1 v1", "p3 s0", "w2 s1 k2 v2 w3 s2 k3 v3 s3"]),
            8: ("q0", "h0 q1 h1", ["q2 p1 k0 v0", "q3 p2 k1 v1", "p3 s0", "w2 s1 k2 v2 w3 s2 k3 v3 s3"]),
            5: ("q0 q1 p0", "", ["q2 p1 k0 v0", "q3 p2 k1 v1", "p3 s0", "w2 s1 k2 v2 w3 s2 k3 v3 s3"]),
            4: ("q0", "q1 p0 q2", ["p1 k0 v0", "q3 p2 s0 k1 v1", "p3 w2 s1", "k2 v2 w3 s2 k3 v3 s3"]),
        }[sched]
        def issue(names):
            for nm in names.split():
                cp(nm).start()
        issue(SCH[0])
        def early(i):
            issue(SCH[2][i])

        def col_prep():
            rows = jnp.concatenate([shift_ref[...].astype(f32), dd_ref[...].astype(f32).reshape(1, D), jnp.zeros((3, D), f32)], axis=0)
            colT = jnp.concatenate([rows, jnp.zeros((120, D), f32)], axis=0).T
            for j in range(5):
                col_ref[j] = jnp.broadcast_to(colT[:, j:j + 1], (D, P))
        zero_ref[0] = 0
        if colpos == 0:
            with scope('col'):
                col_prep()

        def compute_kv(r0, CG=CG):
            kk = ldp(k_buf, r0, CG, 0, S)
            kpad = jnp.concatenate([jnp.zeros((CG, P), bf16), kk], axis=1)
            ks = None
            for j in range(4):
                w = jnp.concatenate([col_ref[j, pl.ds(r0, CG), :]] * (S // P), axis=1)
                kj = kk if j == 0 else kpad[:, P - j:P - j + S]
                t = kj.astype(f32) * w
                ks = t if ks is None else ks + t
            stp(kvT, r0, CG, 0, S, (ks * ldp(v_buf, r0, CG, 0, S).astype(f32)).astype(bf16))

        lane1 = jax.lax.broadcasted_iota(jnp.int32, (1, P), 1)
        sgn = jnp.where(lane1 % 2 == 0, 1.0, -1.0).astype(f32)

        XO, KO, ZO = 0, A * CG, 2 * A * CG
        def c3(zdyn, glo=0, ghi=CG):
            for g0 in range(glo, ghi, RG):
                ldx = lambda a, h: wk_ref[pl.ds(XO + a * CG + g0, RG), h * P:(h + 1) * P]
                ldk = lambda a, h: wk_ref[pl.ds(KO + a * CG + g0, RG), h * P:(h + 1) * P]
                for m in range(A - 1, 0, -1):
                    kr = ldk(m, 0) - sgn * ldk(m - 1, 1)
                    ki = ldk(m, 1) + sgn * ldk(m - 1, 0)
                    wk_ref[pl.ds(KO + m * CG + g0, RG), 0:P] = kr
                    wk_ref[pl.ds(KO + m * CG + g0, RG), P:2 * P] = ki
                for a0 in range(0, A, AG):
                    zr = [None] * AG; zi = [None] * AG
                    xw = {}
                    for m in range(a0 + AG):
                        kr = ldk(m, 0); ki = ldk(m, 1)
                        for t in range(AG):
                            a = a0 + t
                            if m > a: continue
                            b = a - m
                            if b not in xw:
                                xw[b] = (ldx(b, 0), ldx(b, 1))
                            xr, xi = xw[b]
                            tr = kr * xr - ki * xi
                            ti = kr * xi + ki * xr
                            zr[t] = tr if zr[t] is None else zr[t] + tr
                            zi[t] = ti if zi[t] is None else zi[t] + ti
                    for t in range(AG):
                        a = a0 + t
                        zrow = ZO + (a * CG + g0) // 2
                        if alias:
                            zrow = pl.multiple_of(zdyn + zrow, 8)
                        wk_ref[pl.ds(zrow, RG // 2), 0:P] = pltpu.bitcast(zr[t].astype(bf16), f32)
                        wk_ref[pl.ds(zrow, RG // 2), P:2 * P] = pltpu.bitcast(zi[t].astype(bf16), f32)

        def conv_fwd(r0):
            lx = jnp.concatenate([ldp(kvT, r0, CG, a * P, P) for a in range(A)], axis=0)
            lk = jnp.concatenate([ldp(ssm_buf, r0, CG, a * P, P) for a in range(A)], axis=0)
            wk_ref[pl.ds(XO, A * CG), :] = jnp.dot(lx, ft_ref[...], preferred_element_type=f32)
            wk_ref[pl.ds(KO, A * CG), :] = jnp.dot(lk, ft_ref[...], preferred_element_type=f32)
        def conv_inv(r0):
            yb = jnp.dot(pltpu.bitcast(wk_ref[pl.ds(ZO, A * CG // 2), :], bf16), g_ref[...], preferred_element_type=f32)
            for a in range(A):
                y_ref[pl.ds(r0, CG), a * P:(a + 1) * P] = yb[a * CG:(a + 1) * CG, :]
        def bias1(off):
            return b1_ref[pl.ds(off, FC)].astype(f32).reshape(1, FC)

        def act(j, slot):
            off = pl.multiple_of(j * FC, FC)
            stp(u_ref, 0, D, off, FC, gelu(pre_ref[slot] + bias1(off)).astype(bf16))

        def ln_chunk(i, LNC=LNC):
            for t in range(QC // LNC):
                off = i * QC + t * LNC if isinstance(i, int) else pl.multiple_of(i * QC + t * LNC, LNC)
                xt = ldp(xT, 0, D, off, LNC).astype(f32)
                xn = ln0(xt).astype(bf16)
                stp(xnT, 0, D, off, LNC, xn)
                stp(hT, 0, D, off, LNC, ln0(xn.astype(f32)).astype(bf16))
        assert NQ == 4
        with scope('ln0'):
            q_copy(0).wait()
            issue(SCH[1])
            ln_chunk(0)
            if colpos == 1:
                col_prep()
        F0 = 2 * FC
        def kslice(c):
            off = c * QC
            if c < NQ - 1:
                q_copy(c + 1).wait()
            if c == 1:
                k_copy(0).wait(); v_copy(0).wait()
            if c == (2 if cv == 0 else 3):
                ssm_copy(0).wait()
            if c == (3 if cv == 0 else 2):
                k_copy(1).wait(); v_copy(1).wait()
            if c == 0 and split0:
                w1h_copy(1).wait()
                pre_ref[1] = jnp.dot(ldp(hT, 0, D, 0, QC), ldp(w1_buf, 0, QC, FC, FC), preferred_element_type=f32)
                ln_chunk(1, LNI)
                return
            w1p_copy(c).wait()
            lhs = ldp(hT, 0, D, off, QC)
            if c == (2 if cv == 0 else 3):
                conv_fwd(0)
            pab = jnp.dot(lhs, ldp(w1_buf, off, QC, 0, F0), preferred_element_type=f32)
            pa = pab[:, 0:FC]
            pb = pab[:, FC:F0]
            if c < NQ - 1:
                ln_chunk(c + 1, LNI)
            if c == 1:
                compute_kv(0)
            if c == 2 and cv == 0:
                c3(zero_ref[0], 0, CG // 2)
            if c == 2 and cv == 1:
                compute_kv(CG)
            if c == 0:
                pre_ref[0] = pa
                pre_ref[1] = pb
            elif c < NQ - 1:
                pre_ref[0] += pa
                pre_ref[1] += pb
            else:
                c3(zero_ref[0], CG // 2 if cv == 0 else 0, CG)
                if cv == 0:
                    compute_kv(CG)
                stp(u_ref, 0, D, 0, FC, gelu(pre_ref[0] + pa + bias1(0)).astype(bf16))
                pre_ref[1] += pb
                conv_inv(0)
        if split0:
            @pl.when(zero_ref[0] == 0)
            def _():
                w1h_copy(0).wait()
                pre_ref[0] = jnp.dot(ldp(hT, 0, D, 0, QC), ldp(w1_buf, 0, QC, 0, FC), preferred_element_type=f32)
        def cbody(c, carry):
            for i in range(NQ):
                pl.when(c == i)(functools.partial(early, i))
            for i in range(NQ):
                pl.when(c == i)(functools.partial(kslice, i))
            return carry
        with scope('cloop'):
            jax.lax.fori_loop(0, NQ, cbody, 0)


        def bodyA(j, c):
            off = pl.multiple_of(j * FC, FC)
            r0 = pl.multiple_of((j - 1) * CG, CG)
            @pl.when(j + 2 < NJ)
            def _():
                w1_copy(j + 2).start()
                k_copy(j + 2).start(); v_copy(j + 2).start(); ssm_copy(j + 2).start()
            @pl.when(j >= NJ - W2E)
            def _():
                w2_copy(j - (NJ - W2E), 0).start(); w2_copy(j - (NJ - W2E), 1).start()
            k_copy(j).wait(); v_copy(j).wait()
            w1_copy(j).wait()
            ssm_copy(j - 1).wait()
            slot = j % 2
            conv_fwd(r0)
            u = jnp.dot(ldp(hT, 0, D, 0, S), ldp(w1_buf, 0, S, off, FC), preferred_element_type=f32)
            c3(jnp.minimum(j, 0))
            act(j - 1, 1 - slot)
            conv_inv(r0)
            compute_kv(pl.multiple_of(j * CG, CG))
            pre_ref[slot] = u
            return c
        with scope('phaseA'):
            jax.lax.fori_loop(2, NJ, bodyA, 0)

        def epilogue(n, slot):
            off = pl.multiple_of(n * NC, NC)
            yy = acc_ref[slot] + b2_ref[pl.ds(off, NC)].astype(f32).reshape(1, NC)
            g = silu(yy)
            dc = jnp.concatenate([col_ref[4]] * (NC // P), axis=1)
            yv = y_ref[:, pl.ds(off, NC)] + ldp(kvT, 0, D, off, NC).astype(f32) * dc
            o = ldp(xT, 0, D, off, NC).astype(f32) + ldp(xnT, 0, D, off, NC).astype(f32) * yv * g
            stp(out_buf, 0, D, off, NC, o.astype(bf16))
        def mm2(off):
            return (jnp.dot(ldp(u_ref, 0, D, 0, KH), ldp(w2a_buf, 0, KH, off, NC), preferred_element_type=f32)
                    + jnp.dot(ldp(u_ref, 0, D, KH, KH), ldp(w2b_buf, 0, KH, off, NC), preferred_element_type=f32))

        with scope('B0'):
            w2_copy(W2E, 0).start(); w2_copy(W2E, 1).start()
            ssm_copy(NG - 1).wait()
            w2_copy(0, 0).wait(); w2_copy(0, 1).wait()
            rl = (NG - 1) * CG
            conv_fwd(rl)
            KL = F - FC
            part = (jnp.dot(ldp(u_ref, 0, D, 0, KH), ldp(w2a_buf, 0, KH, 0, NC), preferred_element_type=f32)
                    + jnp.dot(ldp(u_ref, 0, D, KH, KL - KH), ldp(w2b_buf, 0, KL - KH, 0, NC), preferred_element_type=f32))
            c3(zero_ref[0])
            act(NJ - 1, (NJ - 1) % 2)
            part = part + jnp.dot(ldp(u_ref, 0, D, KL, FC), ldp(w2b_buf, KL - KH, FC, 0, NC), preferred_element_type=f32)
            conv_inv(rl)
            acc_ref[0] = part

        def bodyB(n, c):
            off = pl.multiple_of(n * NC, NC)
            @pl.when(n + W2E < NN)
            def _():
                w2_copy(n + W2E, 0).start(); w2_copy(n + W2E, 1).start()
            @pl.when(n >= 2)
            def _():
                o_copy(n - 2).start()
            w2_copy(n, 0).wait(); w2_copy(n, 1).wait()
            slot = n % 2
            epilogue(n - 1, 1 - slot)
            acc_ref[slot] = mm2(off)
            return c
        with scope('phaseB'):
            jax.lax.fori_loop(1, NN, bodyB, 0)
        with scope('tail'):
            o_copy(NN - 2).start()
            epilogue(NN - 1, (NN - 1) % 2)
            o_copy(NN - 1).start()
            for n in range(NN):
                o_copy(n).wait()

    def fn(A_q, A_k, A_v, A_shift_k, A_ssm_k, A_ssm_D, B_x, B_w1, B_b1, B_w2, B_b2):
        any_spec = pl.BlockSpec(memory_space=pltpu.HBM)
        vm = pl.BlockSpec(memory_space=pltpu.VMEM)
        outT = pl.pallas_call(
            kernel,
            out_shape=jax.ShapeDtypeStruct((1, D, S), bf16),
            in_specs=[any_spec, any_spec, any_spec, vm, any_spec, vm, any_spec, vm, any_spec, vm, vm, vm],
            out_specs=any_spec,
            scratch_shapes=[
                pltpu.VMEM((D // 2, S), jnp.uint32), pltpu.VMEM((D // 2, S), jnp.uint32), pltpu.VMEM((D // 2, S), jnp.uint32), pltpu.VMEM((D // 2, S), jnp.uint32),
                pltpu.VMEM((S // 2, F), jnp.uint32), pltpu.VMEM((F // 4, S), jnp.uint32), pltpu.VMEM((F // 4, S), jnp.uint32),
                pltpu.VMEM((D // 2, S), jnp.uint32), pltpu.VMEM((D // 2, S), jnp.uint32), pltpu.VMEM((D // 2, S), jnp.uint32),
                pltpu.VMEM((D, S), f32), pltpu.VMEM((D // 2, F), jnp.uint32), pltpu.VMEM((D // 2, S), jnp.uint32),
                pltpu.VMEM((2 * A * CG + A * CG // 2, 2 * P), f32), pltpu.VMEM((2, D, FC), f32), pltpu.SMEM((1,), jnp.int32),
                pltpu.VMEM((5, D, P), f32), pltpu.VMEM((2, D, NC), f32),
                pltpu.SemaphoreType.DMA((NQ,)), pltpu.SemaphoreType.DMA((NG,)), pltpu.SemaphoreType.DMA((NG,)), pltpu.SemaphoreType.DMA((NG,)),
                pltpu.SemaphoreType.DMA((NJ,)), pltpu.SemaphoreType.DMA((NQ,)), pltpu.SemaphoreType.DMA((2 * NN,)), pltpu.SemaphoreType.DMA((NN,)),
            ],
            compiler_params=pltpu.CompilerParams(vmem_limit_bytes=vmem * 1024 * 1024, flags=flags, disable_bounds_checks=nobc),
        )(A_q.transpose(0, 2, 1), A_k.transpose(0, 2, 1), A_v.transpose(0, 2, 1), A_shift_k.T, A_ssm_k,
          A_ssm_D, B_w1, B_b1, B_w2, B_b2, FT_NP, G_NP)
        return outT.transpose(0, 2, 1)
    return fn


_KERNEL_FN = make()


@jax.jit
def pallas_recurrent_scan__ssm_conv_h3__mixer_token_mlp__prompt_kernel(
    A_q: jax.Array,
    A_k: jax.Array,
    A_v: jax.Array,
    A_shift_k: jax.Array,
    A_ssm_k: jax.Array,
    A_ssm_D: jax.Array,
    B_x: jax.Array,
    B_w1: jax.Array,
    B_b1: jax.Array,
    B_w2: jax.Array,
    B_b2: jax.Array,
):
    return _KERNEL_FN(A_q, A_k, A_v, A_shift_k, A_ssm_k, A_ssm_D, B_x, B_w1, B_b1, B_w2, B_b2)
```
